```python
import os as _os
_os.environ.setdefault("JAX_PLATFORMS", "cpu")
import jax
import jax.numpy as jnp

def _softmax(x, axis=-1):
    return jax.nn.softmax(x, axis=axis)
def _gelu(x):
    return jax.nn.gelu(x, approximate=True)
def _silu(x):
    return jax.nn.silu(x)
def _sigmoid(x):
    return jax.nn.sigmoid(x)
def _layernorm(x, axis=-1, eps=1e-5):
    m = jnp.mean(x, axis=axis, keepdims=True)
    v = jnp.var(x, axis=axis, keepdims=True)
    return (x - m) / jnp.sqrt(v + eps)
def _scatter_add(tgt, idx, src, axis=0):
    return tgt.at[idx].add(src)
def _segment_sum(src, seg, n):
    return jax.ops.segment_sum(src, seg, n)
class _Rng:
    def __init__(self, key):
        self._k = key
    def _next(self):
        self._k, sub = jax.random.split(self._k)
        return sub
    def normal(self, shape):
        return jax.random.normal(self._next(), shape, dtype=jnp.bfloat16)
    def randint(self, lo, hi, shape):
        return jax.random.randint(self._next(), shape, lo, hi, dtype=jnp.int32)
    def uniform(self, shape, lo=0.0, hi=1.0):
        return jax.random.uniform(self._next(), shape, jnp.bfloat16, lo, hi)
    def permutation(self, n):
        return jax.random.permutation(self._next(), n)


kernel_name = 'parallel_sum__mha_block__swiglu_ffn__prompt'

def setup_inputs():
    _rng = _Rng(jax.random.key(int.from_bytes(__import__("os").urandom(4), "little")))
    _w = (lambda a: (lambda t: t.astype(jnp.bfloat16) if jnp.issubdtype(t.dtype, jnp.floating) else t)(jnp.asarray(a)))
    def _A_setup():
        B, S, D, H = 1, 2048, 640, 32
        return {
            "x": _w((lambda *s: _rng.normal(s) * 0.05)(B, S, D)),
            "wqkv": _w((lambda *s: _rng.normal(s) * 0.1)(D, 3 * D)),
            "wo": _w((lambda *s: _rng.normal(s) * 0.05)(D, D)),
        }
    _A_in = _A_setup()

    def _B_setup():
        B, S, D, F = 1, 2048, 640, 1536
        return {
            "x": _w((lambda *s: _rng.normal(s) * 0.05)(B, S, D)),
            "w_gate": _w((lambda *s: _rng.normal(s) * 0.05)(D, F)),
            "w_up": _w((lambda *s: _rng.normal(s) * 0.05)(D, F)),
            "w_down": _w((lambda *s: _rng.normal(s) * 0.05)(F, D)),
        }
    _B_in = _B_setup()

    return {
        "A_x": _A_in["x"],
        "A_wqkv": _A_in["wqkv"],
        "A_wo": _A_in["wo"],
        "B_x": _B_in["x"],
        "B_w_gate": _B_in["w_gate"],
        "B_w_up": _B_in["w_up"],
        "B_w_down": _B_in["w_down"],
    }

def reference(A_x, A_wqkv, A_wo, B_x, B_w_gate, B_w_up, B_w_down):
    def _A_ref(x, wqkv, wo):
        B, S, D = x.shape
        H = 32
        Dh = D // H
        qkv = (lambda x, *d: x.transpose(*d))((x @ wqkv).reshape(B, S, 3, H, Dh), 2, 0, 3, 1, 4)
        q, k, v = qkv[0], qkv[1], qkv[2]
        scores = jnp.einsum("bhqd,bhkd->bhqk", q, k) * (Dh ** -0.5)
        p = _softmax(scores, axis=-1)
        o = jnp.einsum("bhqk,bhkd->bhqd", p, v)
        return (lambda x, *d: x.transpose(*d))(o, 0, 2, 1, 3).reshape(B, S, D) @ wo

    def _B_ref(x, w_gate, w_up, w_down):
        g = _silu(x @ w_gate)
        u = x @ w_up
        return (g * u) @ w_down

    x = A_x
    xn = _layernorm(x, axis=-1)
    return x + _A_ref(xn, A_wqkv, A_wo) + _B_ref(xn, B_w_gate, B_w_up, B_w_down)
```

```python
import functools
import math

import jax
import jax.numpy as jnp
from jax import lax
from jax.experimental import pallas as pl
from jax.experimental.pallas import tpu as pltpu

F32, BF16, U32 = jnp.float32, jnp.bfloat16, jnp.uint32
S, D, H, DH, F = 2048, 640, 32, 20, 1536
TQ = 512
NB = S // TQ
CK = 128
NCH = D // 128
QSCALE = (DH ** -0.5) * math.log2(math.e)


def _dot(a, b):
    return jnp.dot(a, b, preferred_element_type=F32)


def _kernel(x_hbm, wqkv_hbm, wo_hbm, wg_hbm, wu_hbm, wd_hbm, out_hbm,
            x_s, wqkv_s, wo_s, wg_s, wu_s, wd_s, out_s,
            xn_s, qt_s, k_s, vt_s, w_s, s_s, ot_s, in_sem, out_sem, *, UQ):
    def x_copy(b):
        return pltpu.make_async_copy(x_hbm.at[pl.ds(b * TQ, TQ)], x_s.at[b], in_sem.at[b])

    def wqkv_copy(j):
        return pltpu.make_async_copy(wqkv_hbm.at[:, pl.ds(j * D, D)], wqkv_s.at[j], in_sem.at[NB + j])

    late = [pltpu.make_async_copy(src, dst, in_sem.at[NB + 3 + i])
            for i, (src, dst) in enumerate(((wg_hbm, wg_s), (wu_hbm, wu_s), (wo_hbm, wo_s), (wd_hbm, wd_s)))]

    x_copy(0).start()
    for j in range(3):
        wqkv_copy(j).start()
    for b in range(1, NB):
        x_copy(b).start()
    for c in late:
        c.start()
    for j in range(3):
        wqkv_copy(j).wait()

    def proj(b, carry):
        x_copy(b).wait()
        x = x_s[b].astype(F32)
        mu = jnp.mean(x, axis=-1, keepdims=True)
        xc = x - mu
        var = jnp.mean(xc * xc, axis=-1, keepdims=True)
        xn = (xc * lax.rsqrt(var + 1e-5)).astype(BF16)
        xn_s[b] = pltpu.bitcast(xn, U32)

        q = _dot(xn, wqkv_s[0]) * QSCALE
        qt_s[b] = pltpu.bitcast(q.T.astype(BF16), U32)

        v = _dot(xn, wqkv_s[2])
        vt = v.T
        lo = lax.broadcasted_iota(jnp.int32, (8, TQ), 0) < 4
        for p in range(H // 2):
            r = 40 * p
            mid = vt[r + 16:r + 24]
            vt_s[p, b, 0:16] = vt[r:r + 16]
            vt_s[p, b, 16:24] = jnp.where(lo, mid, 1.0)
            vt_s[p, b, 24:32] = jnp.where(lo, 1.0, mid)
            vt_s[p, b, 32:48] = vt[r + 24:r + 40]

        k = pltpu.bitcast(_dot(xn, wqkv_s[1]).astype(BF16), U32)
        rows = pl.ds(pl.multiple_of(b * (TQ // 2), TQ // 2), TQ // 2)
        hi = lax.broadcasted_iota(jnp.int32, (TQ // 2, 128), 1) >= 64
        for c in range(NCH):
            k_s[c, rows] = k[:, c * 128:(c + 1) * 128]
        for c in range(NCH - 1):
            k_s[NCH + c, rows] = jnp.where(hi, k[:, c * 128:(c + 1) * 128], k[:, (c + 1) * 128:(c + 2) * 128])
        return carry

    lax.fori_loop(0, NB, proj, 0)

    def prep_w(h, qb, slot):
        lo = h * (DH // 2)
        a = lo // 64
        b = (lo + DH // 2 - 1) // 64
        r = lax.broadcasted_iota(jnp.int32, (64, TQ), 0)
        ra = r + (a * 64 - lo)
        rb = r + (b * 64 - lo)
        qa = qt_s[qb, pl.ds(pl.multiple_of(a * 64, 64), 64), :]
        qb_ = qt_s[qb, pl.ds(pl.multiple_of(b * 64, 64), 64), :]
        w = jnp.where((ra >= 0) & (ra < DH // 2), qa,
                      jnp.where((rb >= 0) & (rb < DH // 2), qb_, jnp.zeros_like(qa)))
        w_s[slot] = w

    def kchunk(h):
        lo = h * (DH // 2)
        a = lo // 64
        b = (lo + DH // 2 - 1) // 64
        return jnp.where(a == b, a, NCH + a)

    def qk(kc, wslot, par, c, mx):
        w = pltpu.bitcast(w_s[wslot], BF16)
        kk = pltpu.bitcast(k_s[kc, c * CK // 2:(c + 1) * CK // 2, :], BF16)
        s = _dot(kk, w)
        s_s[par, c * CK:(c + 1) * CK, :] = s
        t = jnp.max(s.reshape(CK // 8, 8, TQ), axis=0)
        return t if mx is None else jnp.maximum(mx, t)

    def pv(p, j, par, c, mb, acc):
        s = s_s[par, c * CK:(c + 1) * CK, :]
        e = jnp.exp2(s.reshape(CK // 8, 8, TQ) - mb[None]).reshape(CK, TQ)
        kb, off = divmod(c * CK, TQ)
        t = _dot(vt_s[p, kb, 24 * j:24 * j + 24, off:off + CK], e)
        return t if acc is None else acc + t

    def finish_max(mx):
        return jnp.broadcast_to(jnp.max(mx, axis=0, keepdims=True), (8, TQ))

    NU = 2 * UQ
    NIT = (H // 2) * NB // UQ

    def unit_id(i, u):
        di, u = divmod(u, NU)
        g = jnp.minimum(i + di, NIT - 1) * UQ + u // 2
        return (g // NB) * 2 + u % 2, g % NB

    for u in range(2):
        prep_w(*unit_id(0, u), u)
    mx = None
    for c in range(S // CK):
        mx = qk(0, 0, 0, c, mx)
    mb0 = finish_max(mx)

    def attn(i, mb):
        lo = lax.broadcasted_iota(jnp.int32, (8, TQ), 0) < 4
        for u in range(NU):
            h, qb = unit_id(i, u)
            hn, _ = unit_id(i, u + 1)
            kc = kchunk(hn)
            p = h // 2
            j = u % 2
            prep_w(*unit_id(i, u + 2), j)
            mx = acc = None
            for c in range(S // CK):
                mx = qk(kc, 1 - j, 1 - j, c, mx)
                acc = pv(p, j, j, c, mb, acc)
            mb = finish_max(mx)
            r0 = pl.multiple_of(p * 40, 8)
            if j == 0:
                inv = 1.0 / acc[20:21]
                o0 = acc * inv
                ot_s[qb, pl.ds(r0, 16), :] = o0[0:16]
                mid = o0[16:24]
            else:
                inv = 1.0 / acc[0:1]
                o1 = acc * inv
                ot_s[qb, pl.ds(r0 + 16, 8), :] = jnp.where(lo, mid, o1[0:8])
                ot_s[qb, pl.ds(r0 + 24, 16), :] = o1[8:24]
        return mb

    lax.fori_loop(0, NIT, attn, mb0)

    for c in late:
        c.wait()

    def out_copy(b):
        return pltpu.make_async_copy(out_s.at[b], out_hbm.at[pl.ds(b * TQ, TQ)], out_sem.at[b])

    def tail(b, carry):
        xn = pltpu.bitcast(xn_s[b], BF16)
        g = _dot(xn, wg_s[...])
        u = _dot(xn, wu_s[...])
        hid = (g * jax.nn.sigmoid(g) * u).astype(BF16)
        o = ot_s[b].T.astype(BF16)
        y = x_s[b].astype(F32) + _dot(o, wo_s[...]) + _dot(hid, wd_s[...])
        out_s[b] = y.astype(BF16)
        out_copy(b).start()
        return carry

    lax.fori_loop(0, NB, tail, 0)
    for b in range(NB):
        out_copy(b).wait()


@jax.jit
def pallas_parallel_sum__mha_block__swiglu_ffn__prompt_kernel(
    A_x, A_wqkv, A_wo, B_x, B_w_gate, B_w_up, B_w_down,
):
    del B_x
    any_spec = pl.BlockSpec(memory_space=pl.ANY)
    out = pl.pallas_call(
        functools.partial(_kernel, UQ=2),
        out_shape=jax.ShapeDtypeStruct((S, D), BF16),
        in_specs=[any_spec] * 6,
        out_specs=any_spec,
        scratch_shapes=[
            pltpu.VMEM((NB, TQ, D), BF16),
            pltpu.VMEM((3, D, D), BF16),
            pltpu.VMEM((D, D), BF16),
            pltpu.VMEM((D, F), BF16),
            pltpu.VMEM((D, F), BF16),
            pltpu.VMEM((F, D), BF16),
            pltpu.VMEM((NB, TQ, D), BF16),
            pltpu.VMEM((NB, TQ // 2, D), U32),
            pltpu.VMEM((NB, D // 2, TQ), U32),
            pltpu.VMEM((2 * NCH - 1, S // 2, 128), U32),
            pltpu.VMEM((H // 2, NB, 48, TQ), F32),
            pltpu.VMEM((2, 64, TQ), U32),
            pltpu.VMEM((2, S, TQ), F32),
            pltpu.VMEM((NB, D, TQ), F32),
            pltpu.SemaphoreType.DMA((NB + 7,)),
            pltpu.SemaphoreType.DMA((NB,)),
        ],
        compiler_params=pltpu.CompilerParams(vmem_limit_bytes=100 << 20),
        name="fused_block",
    )(A_x.reshape(S, D), A_wqkv, A_wo, B_w_gate, B_w_up, B_w_down)
    return out.reshape(1, S, D)
```

```python
import math

import jax
import jax.numpy as jnp
from jax import lax
from jax.experimental import pallas as pl
from jax.experimental.pallas import tpu as pltpu

F32, BF16, U32 = jnp.float32, jnp.bfloat16, jnp.uint32
S, D, H, DH, F = 2048, 640, 32, 20, 1536
TQ = 512
NB = S // TQ
NT = TQ // 128
CK = 128
NC = S // CK
NCH = D // 128
WQ = D - 128
RO = 256
G = 16
VKEYS = tuple(G * int(c) for c in "1111011110111110")
VOFF = tuple(sum(VKEYS[:c]) for c in range(NC + 1))
QSCALE = (DH ** -0.5) * math.log2(math.e)


def _dot(a, b):
    return jnp.dot(a, b, preferred_element_type=F32)


def _rows8(x):
    return x.reshape(x.shape[0] // 8, 8, x.shape[1])


def _head_words(h):
    lo = h * (DH // 2)
    return lo, lax.shift_right_logical(lo, 6), lax.shift_right_logical(lo + DH // 2 - 1, 6)


def _kchunk(h):
    _, a, b = _head_words(h)
    return jnp.where(a == b, a, NCH + a)


def _never(words):
    return (words | 1) == 0


def _tile_placement():
    rows = [(c, r) for c in range(NC) for r in range(VKEYS[c], CK, 8)]
    tiles = [(c, g, q) for c in range(NC) for g in range(0, VKEYS[c], G) for q in range(NT)]
    where = {}
    for n, tile in enumerate(tiles):
        due = (n + 0.5) * len(rows) / len(tiles)
        at = next(row for i, row in enumerate(rows) if i + 1 >= due and row[0] >= tile[0])
        where.setdefault(at, []).append(tile)
    return where


def _kernel(x_hbm, wqkv_hbm, wo_hbm, wg_hbm, wu_hbm, wd_hbm, out_hbm,
            wo_s, y_s, qt_s, qf_s, k_s, kb_s, vt_s, wo_sem):
    wo_copy = pltpu.make_async_copy(wo_hbm, wo_s, wo_sem)

    def dense(x_s, wqkv_s, wg_s, wu_s, wd_s, xn_s, sem):
        x_copy = [pltpu.make_async_copy(x_hbm.at[pl.ds(b * TQ, TQ)], x_s.at[b], sem.at[b])
                  for b in range(NB)]
        wq_copy, wk_copy, wv_copy = (
            pltpu.make_async_copy(wqkv_hbm.at[:, pl.ds(j * D, D)], wqkv_s.at[j], sem.at[NB + j])
            for j in range(3))
        ffn_copy = [pltpu.make_async_copy(src, dst, sem.at[NB + 3 + i])
                    for i, (src, dst) in enumerate(((wg_hbm, wg_s), (wu_hbm, wu_s), (wd_hbm, wd_s)))]
        for c in (x_copy[0], wk_copy, wq_copy, x_copy[1], wv_copy, x_copy[2], x_copy[3],
                  *ffn_copy, wo_copy):
            c.start()

        def norm(b, during=None):
            x = x_s[b].astype(F32)
            if during is not None:
                pins = []
                for r in range(TQ // 8):
                    t, o = divmod(3 * r, TQ // 8)
                    pins.append(during[8 * o:8 * o + 8, t * 128:(t + 1) * 128])
                x0 = jnp.where(_never(xn_s[0, 0:8, 0:128])[None], jnp.stack(pins), _rows8(x[:, 0:128]))
                x = jnp.concatenate([x0.reshape(TQ, 128), x[:, 128:]], axis=1)
            xc = x - jnp.mean(x, axis=-1, keepdims=True)
            var = jnp.mean(xc * xc, axis=-1, keepdims=True)
            xn_s[b] = pltpu.bitcast((xc * lax.rsqrt(var + 1e-5)).astype(BF16), U32)

        def proj_q(b, norm_next=False):
            q = _dot(pltpu.bitcast(xn_s[b], BF16), wqkv_s[0])
            if norm_next:
                norm(b + 1, q)
            q = (q * QSCALE).T
            qt_s[b] = pltpu.bitcast(q.astype(BF16), U32)
            for p in range(H // 2):
                r = 2 * DH * p
                qf_s[b, 2 * p] = q[r:r + 24]
                qf_s[b, 2 * p + 1, 0:16] = q[r + 24:r + 40]
                qf_s[b, 2 * p + 1, 16:24] = pltpu.roll(q[r + 16:r + 24], 4, 0)

        def proj_v(b):
            vt = _dot(pltpu.bitcast(xn_s[b], BF16), wqkv_s[2]).T
            lo = lax.broadcasted_iota(jnp.int32, (8, TQ), 0) < 4
            for p in range(H // 2):
                r = 2 * DH * p
                mid = vt[r + 16:r + 24]
                vt_s[2 * p, b, 0:16] = vt[r:r + 16]
                vt_s[2 * p, b, 16:24] = jnp.where(lo, mid, 1.0)
                vt_s[2 * p + 1, b, 0:8] = jnp.where(lo, 1.0, mid)
                vt_s[2 * p + 1, b, 8:24] = vt[r + 24:r + 40]

        def proj_k(b):
            xn = pltpu.bitcast(xn_s[b], BF16)
            edge = jnp.concatenate(
                [_dot(xn[r:r + 128, WQ:], wqkv_s[1, WQ:, WQ:]) for r in range(0, TQ, 128)], axis=0)
            edge = edge + _dot(xn[:, :WQ], wqkv_s[1, :WQ, WQ:])
            k = jnp.concatenate([_dot(xn, wqkv_s[1, :, :WQ]), edge], axis=1)
            k = pltpu.bitcast(k.astype(BF16), U32)
            hi = lax.broadcasted_iota(jnp.int32, (TQ // 2, 128), 1) >= 64
            for c in range(NCH):
                k_s[c, b] = k[:, c * 128:(c + 1) * 128]
            for c in range(NCH - 1):
                k_s[NCH + c, b] = jnp.where(hi, k[:, c * 128:(c + 1) * 128],
                                            k[:, (c + 1) * 128:(c + 2) * 128])

        x_copy[0].wait()
        norm(0)
        wk_copy.wait()
        proj_k(0)
        wq_copy.wait()
        x_copy[1].wait()
        proj_q(0, True)
        proj_k(1)
        wv_copy.wait()
        x_copy[2].wait()
        x_copy[3].wait()
        proj_q(1, True)
        proj_v(0)
        proj_k(2)
        proj_q(2, True)
        proj_v(1)
        proj_v(2)
        proj_q(3)
        proj_v(3)
        proj_k(3)
        for c in ffn_copy:
            c.wait()

        def spread_keys(h, odd):
            rows = []
            for c in range(NC):
                kb, off = divmod(c * CK, TQ)
                if VKEYS[c]:
                    rows.append(k_s[_kchunk(h), kb, off // 2:(off + VKEYS[c]) // 2, :])
            k = pltpu.roll(jnp.concatenate(rows, axis=0), (-h * DH) & 127, 1)
            for e in range(DH):
                val = jnp.broadcast_to(k[:, e:e + 1], k.shape)
                kb_s[h, (e - 4) % DH if odd else e] = pltpu.bitcast(val, BF16).astype(F32)

        def ffn(b, carry):
            for n in range(H // NB):
                spread_keys(b * (H // NB) + n, n % 2)
            xn = pltpu.bitcast(xn_s[b], BF16)
            half = _dot(xn, wg_s[...]) * 0.5
            gate = half * jnp.tanh(half) + half
            hid = (gate * _dot(xn, wu_s[...])).astype(BF16)
            y_s[b] = x_s[b].astype(F32) + _dot(hid, wd_s[...])
            return carry

        lax.fori_loop(0, NB, ffn, 0)

    pl.run_scoped(
        dense,
        pltpu.VMEM((NB, TQ, D), BF16),
        pltpu.VMEM((3, D, D), BF16),
        pltpu.VMEM((D, F), BF16),
        pltpu.VMEM((D, F), BF16),
        pltpu.VMEM((F, D), BF16),
        pltpu.VMEM((NB, TQ // 2, D), U32),
        pltpu.SemaphoreType.DMA((NB + 6,)),
    )

    def attention(w_s, s_s, m_s, o_s, out_s, sem):
        ot_s = qf_s
        where = _tile_placement()

        def mask_queries(h, qb, slot, r0):
            lo, a, b = _head_words(h)
            r = lax.broadcasted_iota(jnp.int32, (8, TQ), 0) + r0
            ra = r + (a * 64 - lo)
            rb = r + (b * 64 - lo)
            qa = qt_s[qb, pl.ds(pl.multiple_of(a * 64 + r0, 8), 8), :]
            qc = qt_s[qb, pl.ds(pl.multiple_of(b * 64 + r0, 8), 8), :]
            w_s[slot, r0:r0 + 8, :] = jnp.where(
                (ra >= 0) & (ra < DH // 2), qa,
                jnp.where((rb >= 0) & (rb < DH // 2), qc, jnp.zeros_like(qa)))

        def update_max(mx, s, q0):
            for t in range(s.shape[1] // 128):
                x = jnp.max(_rows8(s[:, t * 128:(t + 1) * 128]), axis=0)
                mx[q0 + t] = x if mx[q0 + t] is None else jnp.maximum(mx[q0 + t], x)

        def score(h, qb, slot, c, mx, zero):
            kb, off = divmod(c * CK, TQ)
            a = VKEYS[c]
            k = k_s[_kchunk(h) + zero * qb, kb, (off + a) // 2:(off + CK) // 2, :]
            sm = _dot(pltpu.bitcast(k, BF16), pltpu.bitcast(w_s[slot], BF16))
            s_s[qb, c * CK + a:(c + 1) * CK, :] = sm
            for r in range(a, CK, 8):
                for tc, g, q in where.get((c, r), ()):
                    cols = slice(q * 128, (q + 1) * 128)
                    r0 = VOFF[tc] + g
                    hk, hq = h + zero * (q + NT * qb), h + zero * r0
                    s = None
                    for d in range(DH):
                        t = kb_s[hk, d, r0:r0 + G, :] * qf_s[qb, hq, d:d + 1, cols]
                        s = t if s is None else s + t
                    update_max(mx, s, q)
                    s = jnp.minimum(_rows8(s), mx[q][None]).reshape(G, 128)
                    s_s[qb, tc * CK + g:tc * CK + g + G, cols] = s
                update_max(mx, sm[r - a:r - a + 8], 0)
            if c == NC - 1:
                m = jnp.max(jnp.concatenate(mx, axis=1), axis=0, keepdims=True)
                m_s[qb] = jnp.broadcast_to(m, (8, TQ))

        def probs(qb, c, m):
            return jnp.exp2(_rows8(s_s[qb, c * CK:(c + 1) * CK, :]) - m[None]).reshape(CK, TQ)

        def weigh(h, c, p, acc):
            kb, off = divmod(c * CK, TQ)
            return acc + _dot(vt_s[h, kb, :, off:off + CK], p)

        def first_head(qb, carry):
            zero = lax.shift_right_logical(qb, 12)
            for r0 in range(0, 64, 8):
                mask_queries(0, qb, 1, r0)
            mx = [None] * NT
            for c in range(NC):
                score(0, qb, 1, c, mx, zero)
            return carry

        lax.fori_loop(0, NB, first_head, 0)
        for r0 in range(0, 64, 8):
            mask_queries(1, 0, 0, r0)

        def head(h, carry):
            zero = lax.shift_right_logical(h, 12)
            for qb in range(NB):
                m = m_s[qb]
                mx = [None] * NT
                acc = jnp.full((24, TQ), zero.astype(F32))
                hn = h + 1 if qb + 1 < NB else jnp.minimum(h + 2, H - 1)
                for c in range(NC):
                    p = probs(qb, c, m)
                    if c % 2 == 0:
                        mask_queries(hn, (qb + 1) % NB, (qb + 1) % 2, 4 * c)
                    score(h + 1, qb, qb % 2, c, mx, zero)
                    acc = weigh(h + zero * qb, c, p, acc)
                ot_s[qb, h] = acc
            return carry

        lax.fori_loop(0, H - 1, head, 0)
        wo_copy.wait()

        out_copy = [pltpu.make_async_copy(out_s.at[pl.ds(r, RO)], out_hbm.at[pl.ds(r, RO)], sem.at[r // RO])
                    for r in range(0, S, RO)]
        split = -(-WQ // (2 * DH))

        def normalized(b, pairs):
            lo = lax.broadcasted_iota(jnp.int32, (8, TQ), 0) < 4
            parts = []
            for p in pairs:
                a0, a1 = ot_s[b, 2 * p], ot_s[b, 2 * p + 1]
                o0 = a0 * (1.0 / a0[20:21])
                o1 = a1 * (1.0 / a1[0:1])
                parts += [o0[0:16], jnp.where(lo, o0[16:24], o1[0:8]), o1[8:24]]
            return jnp.concatenate(parts, axis=0)

        def gather_front(b):
            o = normalized(b, range(split))[:WQ]
            o_s[b % 2, :, :WQ] = pltpu.bitcast(o.T.astype(BF16), U32)

        def gather_back(b):
            o = normalized(b, range(split - 1, H // 2))[WQ - D:]
            o_s[b % 2, :, WQ:] = pltpu.bitcast(o.T.astype(BF16), U32)

        def project(b, r0, r1, k0, k1, n0, n1):
            o = pltpu.bitcast(o_s[b % 2, r0 // 2:r1 // 2, k0:k1], BF16)
            t = y_s[b, r0:r1, n0:n1] + _dot(o, wo_s[k0:k1, n0:n1])
            if k1 == D:
                out_s[b * TQ + r0:b * TQ + r1, n0:n1] = t.astype(BF16)
            else:
                y_s[b, r0:r1, n0:n1] = t

        gather_front(0)
        for b in range(NB):
            m = m_s[b]
            acc = jnp.concatenate([jnp.where(_never(qt_s[b, 0:8, :]), m, 0.0)] * 3, axis=0)
            for c in range(NC):
                k, r = divmod(c, NT)
                project(b, 128 * r, 128 * r + 128, 128 * k, 128 * k + 128, 0, WQ)
                acc = weigh(H - 1, c, probs(b, c, m), acc)
            ot_s[b, H - 1] = acc
            gather_back(b)
            if b + 1 < NB:
                gather_front(b + 1)
            project(b, 0, TQ, 0, WQ, WQ, D)
            for r in range(0, TQ, 128):
                project(b, r, r + 128, WQ, D, WQ, D)
            for r in range(0, TQ, RO):
                project(b, r, r + RO, WQ, D, 0, WQ)
                out_copy[(b * TQ + r) // RO].start()
        for c in out_copy:
            c.wait()

    pl.run_scoped(
        attention,
        pltpu.VMEM((2, 64, TQ), U32),
        pltpu.VMEM((NB, S, TQ), F32),
        pltpu.VMEM((NB, 8, TQ), F32),
        pltpu.VMEM((2, TQ // 2, D), U32),
        pltpu.VMEM((S, D), BF16),
        pltpu.SemaphoreType.DMA((S // RO,)),
    )


@jax.jit
def pallas_parallel_sum__mha_block__swiglu_ffn__prompt_kernel(
    A_x: jax.Array,
    A_wqkv: jax.Array,
    A_wo: jax.Array,
    B_x: jax.Array,
    B_w_gate: jax.Array,
    B_w_up: jax.Array,
    B_w_down: jax.Array,
):
    del B_x
    hbm = pl.BlockSpec(memory_space=pl.ANY)
    out = pl.pallas_call(
        _kernel,
        out_shape=jax.ShapeDtypeStruct((S, D), BF16),
        in_specs=[hbm] * 6,
        out_specs=hbm,
        scratch_shapes=[
            pltpu.VMEM((D, D), BF16),
            pltpu.VMEM((NB, TQ, D), F32),
            pltpu.VMEM((NB, D // 2, TQ), U32),
            pltpu.VMEM((NB, H, 24, TQ), F32),
            pltpu.VMEM((2 * NCH - 1, NB, TQ // 2, 128), U32),
            pltpu.VMEM((H, DH, VOFF[-1], 128), F32),
            pltpu.VMEM((H, NB, 24, TQ), F32),
            pltpu.SemaphoreType.DMA(()),
        ],
        compiler_params=pltpu.CompilerParams(vmem_limit_bytes=124 << 20),
        name="fused_block",
    )(A_x.reshape(S, D), A_wqkv, A_wo, B_w_gate, B_w_up, B_w_down)
    return out.reshape(1, S, D)
```

```python
import math

import jax
import jax.numpy as jnp
from jax import lax
from jax.experimental import pallas as pl
from jax.experimental.pallas import tpu as pltpu

F32, BF16, U32 = jnp.float32, jnp.bfloat16, jnp.uint32
S, D, H, DH, F = 2048, 640, 32, 20, 1536
TQ = 512
NB = S // TQ
NT = TQ // 128
CK = 128
CB = TQ // CK
G = 16
NCH = D // 128
WQ = 512
RF = S // H
HB = TQ // RF
RO = 256
FFN_SLOTS = "0111" * 10 + "0111" "0101" * 3
QSCALE = (DH ** -0.5) * math.log2(math.e)


def _dot(a, b):
    return jnp.dot(a, b, preferred_element_type=F32)


def _rows8(x):
    return x.reshape(x.shape[0] // 8, 8, x.shape[1])


def _never(words):
    return (words | 1) == 0


def _ffn_step(slot):
    return FFN_SLOTS[:slot].count("1") if FFN_SLOTS[slot] == "1" else None


def _tile_placement(slot0):
    now, points = 0, []
    for c in range(CB):
        for r in range(G, CK, 8):
            now += 8
            points.append((now, ("score", c, r)))
        if slot0 is not None:
            now += 16
            if _ffn_step(slot0 + c) is not None:
                for r in range(0, RF, 8):
                    now += 8
                    points.append((now, ("ffn", c, r)))
    tiles = [(c, q) for c in range(CB) for q in range(NT)]
    where = {}
    for n, tile in enumerate(tiles):
        due = (n + 1) * now / len(tiles)
        at = next((p for t, p in points if t >= due and p[1] >= tile[0]), points[-1][1])
        where.setdefault(at, []).append(tile)
    return where


def _kernel(x_hbm, wqkv_hbm, wo_hbm, wg_hbm, wu_hbm, wd_hbm, out_hbm,
            x_s, wqkv_s, wo_s, wg_s, wu_s, wd_s, wgu_s, wdp_s, xn_s, gu_s, hid_s, y_s,
            qt_s, qf_s, k_s, kh_s, kb0_s, kb_s, vt_s, s_s, m_s, mrun_s, ot_s, o_s, out_s,
            in_sem, out_sem):
    x_copy = [pltpu.make_async_copy(x_hbm.at[pl.ds(b * TQ, TQ)], x_s.at[b], in_sem.at[b])
              for b in range(NB)]
    wq_copy, wk_copy, wv_copy = (
        pltpu.make_async_copy(wqkv_hbm.at[:, pl.ds(j * D, D)], wqkv_s.at[j], in_sem.at[NB + j])
        for j in range(3))
    late_copy = [pltpu.make_async_copy(src, dst, in_sem.at[NB + 3 + i]) for i, (src, dst) in
                 enumerate(((wg_hbm, wg_s), (wu_hbm, wu_s), (wd_hbm, wd_s), (wo_hbm, wo_s)))]
    for c in (x_copy[0], wk_copy, wq_copy, x_copy[1], wv_copy, x_copy[2], x_copy[3], *late_copy):
        c.start()

    def norm(b, during=None):
        x = x_s[b].astype(F32)
        if during is not None:
            pins = []
            for r in range(TQ // 8):
                t, o = divmod(3 * r, TQ // 8)
                pins.append(during[8 * o:8 * o + 8, t * 128:(t + 1) * 128])
            x0 = jnp.where(_never(xn_s[0, 0:8, 0:128])[None], jnp.stack(pins), _rows8(x[:, 0:128]))
            x = jnp.concatenate([x0.reshape(TQ, 128), x[:, 128:]], axis=1)
        xc = x - jnp.mean(x, axis=-1, keepdims=True)
        var = jnp.mean(xc * xc, axis=-1, keepdims=True)
        xn = pltpu.bitcast((xc * lax.rsqrt(var + 1e-5)).astype(BF16), U32)
        xn_s[b * HB:(b + 1) * HB] = xn.reshape(HB, RF // 2, D)

    def normed(b):
        return pltpu.bitcast(xn_s[b * HB:(b + 1) * HB].reshape(TQ // 2, D), BF16)

    def proj_q(b, norm_next=False):
        q = _dot(normed(b), wqkv_s[0])
        if norm_next:
            norm(b + 1, q)
        q = (q * QSCALE).T
        lo = lax.broadcasted_iota(jnp.int32, (8, TQ), 0) < 4
        for p in range(H // 2):
            r = 2 * DH * p
            even = [q[r:r + 16], jnp.where(lo, q[r + 16:r + 24], 0.0)]
            t = [pltpu.roll(q[i:i + 8], 4, 0) for i in range(r + 16, r + 40, 8)]
            odd = [jnp.where(lo, t[0], t[1]), jnp.where(lo, t[1], t[2]), jnp.where(lo, t[2], 0.0)]
            for h, rows in ((2 * p, even), (2 * p + 1, odd)):
                qf_s[b, h] = jnp.concatenate(rows, axis=0)
                rows = jnp.concatenate(rows + [jnp.zeros((8, TQ), F32)], axis=0)
                qt_s[b, h] = pltpu.bitcast(rows.astype(BF16), U32)

    def proj_v(b):
        vt = _dot(normed(b), wqkv_s[2]).T
        lo = lax.broadcasted_iota(jnp.int32, (8, TQ), 0) < 4
        for p in range(H // 2):
            r = 2 * DH * p
            mid = vt[r + 16:r + 24]
            vt_s[2 * p, b, 0:16] = vt[r:r + 16]
            vt_s[2 * p, b, 16:24] = jnp.where(lo, mid, 1.0)
            vt_s[2 * p + 1, b, 0:8] = jnp.where(lo, 1.0, mid)
            vt_s[2 * p + 1, b, 8:24] = vt[r + 24:r + 40]

    def proj_k(b):
        xn = normed(b)
        edge = jnp.concatenate(
            [_dot(xn[r:r + 128, WQ:], wqkv_s[1, WQ:, WQ:]) for r in range(0, TQ, 128)], axis=0)
        edge = edge + _dot(xn[:, :WQ], wqkv_s[1, :WQ, WQ:])
        k = jnp.concatenate([_dot(xn, wqkv_s[1, :, :WQ]), edge], axis=1)
        k_s[b] = pltpu.bitcast(k.astype(BF16), U32)

    def split_heads(b):
        hi = lax.broadcasted_iota(jnp.int32, (TQ // 2, 128), 1) >= 64
        for h in range(H):
            c, lane = divmod(h * DH, 128)
            k = k_s[b, :, c * 128:(c + 1) * 128]
            if lane + DH > 128:
                k = jnp.where(hi, k, k_s[b, :, (c + 1) * 128:(c + 2) * 128])
            kh_s[h, b] = pltpu.roll(k, 128 - lane, 1) if lane else k

    def spread_keys(dst, h, kb, features, order=lambda k: k):
        k = jnp.concatenate([kh_s[h, kb, c * CK // 2:(c * CK + G) // 2] for c in range(CB)], axis=0)
        k = pltpu.bitcast(order(k), BF16).astype(F32)
        for d in features:
            dst[d] = jnp.broadcast_to(k[:, d:d + 1], k.shape)

    def ffn_steps(i, zero, pack_weights=False):
        half_w = WQ // 2

        def gate_up(n, k):
            rows, cols = slice(k * 64, (k + 1) * 64), slice(n * WQ, (n + 1) * WQ)
            if pack_weights:
                src = slice(k * 128, (k + 1) * 128), slice(n * half_w, (n + 1) * half_w)
                w = jnp.concatenate([wg_s[src], wu_s[src]], axis=1)
                wgu_s[rows, cols] = pltpu.bitcast(w, U32)
            else:
                w = pltpu.bitcast(wgu_s[rows, cols], BF16)
            t = _dot(pltpu.bitcast(xn_s[i + zero * n, :, k * 128:(k + 1) * 128], BF16), w)
            if k > 0:
                t = t + gu_s[...]
            if k < NCH - 1:
                gu_s[...] = t
            else:
                half = t[:, :half_w] * 0.5
                gate = half * jnp.tanh(half) + half
                hid = (gate * t[:, half_w:]).astype(BF16)
                hid_s[n // 2][0, :, n % 2 * half_w:(n % 2 + 1) * half_w] = pltpu.bitcast(hid, U32)
            return t

        def down(k, n):
            rows, cols = slice(k * WQ // 2, (k + 1) * WQ // 2), slice(n * 128, (n + 1) * 128)
            if pack_weights:
                w = wd_s[k * WQ:(k + 1) * WQ, cols]
                wdp_s[rows, cols] = pltpu.bitcast(w, U32)
            else:
                w = pltpu.bitcast(wdp_s[rows, cols], BF16)
            t = _dot(pltpu.bitcast(hid_s[k][zero * n], BF16), w)
            if k > 0:
                t = t + y_s[n][i]
            y_s[n][i] = t
            return t

        return ([(gate_up, n, k) for n in range(2 * F // WQ) for k in range(NCH)]
                + [(down, k, n) for k in range(F // WQ) for n in range(NCH)])

    x_copy[0].wait()
    norm(0)
    wk_copy.wait()
    proj_k(0)
    wq_copy.wait()
    x_copy[1].wait()
    proj_q(0, True)
    proj_k(1)
    wv_copy.wait()
    x_copy[2].wait()
    x_copy[3].wait()
    proj_q(1, True)
    split_heads(0)
    proj_v(0)
    proj_k(2)
    proj_q(2, True)
    split_heads(1)
    proj_v(1)
    proj_k(3)
    for c in late_copy:
        c.wait()
    split_heads(2)
    proj_v(2)
    split_heads(3)
    proj_q(3)
    proj_v(3)
    for kb in range(NB):
        spread_keys(kb0_s.at[kb], 0, kb, range(DH))
    for kb in range(NB - 1):
        spread_keys(kb_s[kb], 1, kb, range(DH))
    for step, a, b in ffn_steps(H - 1, 0, pack_weights=True):
        step(a, b)

    def update_max(mx, s, q0):
        for t in range(s.shape[1] // 128):
            x = jnp.max(_rows8(s[:, t * 128:(t + 1) * 128]), axis=0)
            mx[q0 + t] = x if mx[q0 + t] is None else jnp.maximum(mx[q0 + t], x)

    def vpu_score(keys, h, qb, kb, c, q, mx, zero, after=None):
        cols = slice(q * 128, (q + 1) * 128)
        rows = pl.ds(pl.multiple_of(c * G + zero * (8 * (q + NT * qb)), 8), G)
        hq = h + zero * (c + CB * kb)
        s = None
        for d in range(DH):
            t = keys[d, rows, :] * qf_s[qb, hq, d:d + 1, cols]
            s = t if s is None else s + t
        if after is None:
            update_max(mx, s, q)
            s = jnp.minimum(_rows8(s), mx[q][None]).reshape(G, 128)
        else:
            s = jnp.where(zero > 0, after[None], _rows8(s)).reshape(G, 128)
            update_max(mx, s, q)
        s_s[qb, kb * TQ + c * CK:kb * TQ + c * CK + G, cols] = s

    def score(keys, h, qb, kb, c, mx, zero, where):
        k = kh_s[h + zero * qb, kb, (c * CK + G) // 2:(c + 1) * CK // 2, :]
        qt = jnp.concatenate([pltpu.bitcast(qt_s[qb, h], BF16), jnp.zeros((96, TQ), BF16)], axis=0)
        s = _dot(pltpu.bitcast(k, BF16), qt)
        s_s[qb, kb * TQ + c * CK + G:kb * TQ + (c + 1) * CK, :] = s
        for r in range(G, CK, 8):
            for tile in where.get(("score", c, r), ()):
                vpu_score(keys, h, qb, kb, *tile, mx, zero)
            update_max(mx, s[r - G:r - G + 8], 0)

    def column_max(mx):
        return jnp.broadcast_to(jnp.max(jnp.concatenate(mx, axis=1), axis=0, keepdims=True), (8, TQ))

    def probs(qb, kb, c, m):
        s = s_s[qb, kb * TQ + c * CK:kb * TQ + (c + 1) * CK, :]
        return jnp.exp2(_rows8(s) - m[None]).reshape(CK, TQ)

    def weigh(h, kb, c, p, acc):
        return acc + _dot(vt_s[h, kb, :, c * CK:(c + 1) * CK], p)

    def first_head(qb, carry):
        zero = lax.shift_right_logical(qb, 12)
        mx = [None] * NT
        for kb in range(NB):
            for c in range(CB):
                score(kb0_s.at[kb], 0, qb, kb, c, mx, zero, _tile_placement(None))
        m_s[qb] = column_max(mx)
        return carry

    lax.fori_loop(0, NB, first_head, 0)

    def head(h, carry):
        zero = lax.shift_right_logical(h, 12)
        steps = ffn_steps(h, zero)
        assert len(steps) == FFN_SLOTS.count("1") and len(FFN_SLOTS) == NB * NB * CB
        for kb in range(NB):
            for qb in range(NB):
                slot0 = (kb * NB + qb) * CB
                where = _tile_placement(slot0)
                m = m_s[qb]
                if kb == 0:
                    mx = [None] * NT
                    acc = jnp.full((24, TQ), zero.astype(F32))
                else:
                    mx = [mrun_s[qb, :, q * 128:(q + 1) * 128] for q in range(NT)]
                    acc = ot_s[qb, h]
                for c in range(CB):
                    p = probs(qb, kb, c, m)
                    score(kb_s[kb], h + 1, qb, kb, c, mx, zero, where)
                    if c == 0:
                        pin = pltpu.bitcast(mx[0], U32)[None]
                        spread_keys(kb_s[kb - 1], h + 1 if kb == 0 else jnp.minimum(h + 2, H - 1),
                                    (kb - 1) % NB, range(DH * qb // NB, DH * (qb + 1) // NB),
                                    lambda k: jnp.where(zero > 0, pin, _rows8(k)).reshape(k.shape))
                    acc = weigh(h + zero * qb, kb, c, p, acc)
                    if _ffn_step(slot0 + c) is not None:
                        step, a, b = steps[_ffn_step(slot0 + c)]
                        t = step(a, b)
                        for r in range(0, RF, 8):
                            for tile in where.get(("ffn", c, r), ()):
                                vpu_score(kb_s[kb], h + 1, qb, kb, *tile, mx, zero, t[r:r + 8, 0:128])
                ot_s[qb, h] = acc
                if kb < NB - 1:
                    mrun_s[qb] = jnp.concatenate(mx, axis=1)
                else:
                    m_s[qb] = column_max(mx)
        return carry

    lax.fori_loop(0, H - 1, head, 0)

    out_copy = [pltpu.make_async_copy(out_s.at[pl.ds(r, RO)], out_hbm.at[pl.ds(r, RO)], out_sem.at[r // RO])
                for r in range(0, S, RO)]
    split = -(-WQ // (2 * DH))

    def normalized(b, pairs):
        lo = lax.broadcasted_iota(jnp.int32, (8, TQ), 0) < 4
        parts = []
        for p in pairs:
            a0, a1 = ot_s[b, 2 * p], ot_s[b, 2 * p + 1]
            o0 = a0 * (1.0 / a0[20:21])
            o1 = a1 * (1.0 / a1[0:1])
            parts += [o0[0:16], jnp.where(lo, o0[16:24], o1[0:8]), o1[8:24]]
        return jnp.concatenate(parts, axis=0)

    def gather_front(b):
        o = normalized(b, range(split))[:WQ]
        o_s[b, :, :WQ] = pltpu.bitcast(o.T.astype(BF16), U32)

    def gather_back(b):
        o = normalized(b, range(split - 1, H // 2))[WQ - D:]
        o_s[b, :, WQ:] = pltpu.bitcast(o.T.astype(BF16), U32)

    def project(b, r0, r1, k0, k1, n0, n1):
        o = pltpu.bitcast(o_s[b, r0 // 2:r1 // 2, k0:k1], BF16)
        groups = slice(b * HB + r0 // RF, b * HB + r1 // RF)
        y = jnp.concatenate([y_s[n][groups].reshape(r1 - r0, 128) for n in range(n0 // 128, n1 // 128)],
                            axis=1)
        y = y + _dot(o, wo_s[k0:k1, n0:n1])
        if k1 == D:
            y = y + x_s[b, r0:r1, n0:n1].astype(F32)
            out_s[b * TQ + r0:b * TQ + r1, n0:n1] = y.astype(BF16)
        else:
            for n in range(n0 // 128, n1 // 128):
                y_s[n][groups] = y[:, n * 128 - n0:(n + 1) * 128 - n0].reshape(-1, RF, 128)

    gather_front(0)
    for b in range(NB):
        m = m_s[b]
        acc = jnp.concatenate([jnp.where(_never(qt_s[b, 0, 0:8, :]), m, 0.0)] * 3, axis=0)
        for kb in range(NB):
            for c in range(CB):
                project(b, 128 * c, 128 * c + 128, 128 * kb, 128 * kb + 128, 0, WQ)
                acc = weigh(H - 1, kb, c, probs(b, kb, c, m), acc)
        ot_s[b, H - 1] = acc
        gather_back(b)
        if b + 1 < NB:
            gather_front(b + 1)
        project(b, 0, TQ, 0, WQ, WQ, D)
        for r in range(0, TQ, 128):
            project(b, r, r + 128, WQ, D, WQ, D)
        for r in range(0, TQ, RO):
            project(b, r, r + RO, WQ, D, 0, WQ)
            out_copy[(b * TQ + r) // RO].start()
    for c in out_copy:
        c.wait()


@jax.jit
def pallas_parallel_sum__mha_block__swiglu_ffn__prompt_kernel(
    A_x: jax.Array,
    A_wqkv: jax.Array,
    A_wo: jax.Array,
    B_x: jax.Array,
    B_w_gate: jax.Array,
    B_w_up: jax.Array,
    B_w_down: jax.Array,
):
    del B_x
    hbm = pl.BlockSpec(memory_space=pl.ANY)
    vmem = pltpu.VMEM
    out = pl.pallas_call(
        _kernel,
        out_shape=jax.ShapeDtypeStruct((S, D), BF16),
        in_specs=[hbm] * 6,
        out_specs=hbm,
        scratch_shapes=[
            vmem((NB, TQ, D), BF16),
            vmem((3, D, D), BF16),
            vmem((D, D), BF16),
            vmem((D, F), BF16),
            vmem((D, F), BF16),
            vmem((F, D), BF16),
            vmem((D // 2, 2 * F), U32),
            vmem((F // 2, D), U32),
            vmem((H, RF // 2, D), U32),
            vmem((RF, WQ), F32),
            [vmem((1, RF // 2, WQ), U32)] * (F // WQ),
            [vmem((H, RF, 128), F32)] * NCH,
            vmem((NB, H, 16, TQ), U32),
            vmem((NB, H, 24, TQ), F32),
            vmem((NB, TQ // 2, D), U32),
            vmem((H, NB, TQ // 2, 128), U32),
            vmem((NB, DH, CB * G, 128), F32),
            [vmem((DH, CB * G, 128), F32)] * NB,
            vmem((H, NB, 24, TQ), F32),
            vmem((NB, S, TQ), F32),
            vmem((NB, 8, TQ), F32),
            vmem((NB, 8, TQ), F32),
            vmem((NB, H, 24, TQ), F32),
            vmem((NB, TQ // 2, D), U32),
            vmem((S, D), BF16),
            pltpu.SemaphoreType.DMA((NB + 7,)),
            pltpu.SemaphoreType.DMA((S // RO,)),
        ],
        compiler_params=pltpu.CompilerParams(vmem_limit_bytes=112 << 20),
        name="fused_block",
    )(A_x.reshape(S, D), A_wqkv, A_wo, B_w_gate, B_w_up, B_w_down)
    return out.reshape(1, S, D)
```

```python
import math

import jax
import jax.numpy as jnp
from jax import lax
from jax.experimental import pallas as pl
from jax.experimental.pallas import tpu as pltpu

F32, BF16, U32 = jnp.float32, jnp.bfloat16, jnp.uint32
S, D, H, DH, F = 2048, 640, 32, 20, 1536
TQ = 512
NB = S // TQ
NT = TQ // 128
CK = 128
CB = TQ // CK
G = 16
NCH = D // 128
WQ = 512
RF = S // H
HB = TQ // RF
RO = 256
FFN_SLOTS = "0111" * 10 + "01110101" * 3
QSCALE = (DH ** -0.5) * math.log2(math.e)


def _dot(a, b):
    return jnp.dot(a, b, preferred_element_type=F32)


def _rows8(x):
    return x.reshape(x.shape[0] // 8, 8, x.shape[1])


def _never(words):
    return (words | 1) == 0


def _ffn_step(slot):
    return FFN_SLOTS[:slot].count("1") if FFN_SLOTS[slot] == "1" else None


def _tile_placement(slot0):
    now, points = 0, []
    for c in range(CB):
        for r in range(G, CK, 8):
            now += 8
            points.append((now, ("score", c, r)))
        if slot0 is not None:
            now += 16
            if _ffn_step(slot0 + c) is not None:
                for r in range(0, RF, 8):
                    now += 9
                    points.append((now, ("ffn", c, r)))
    tiles = [(c, q) for c in range(CB) for q in range(NT)]
    where = {}
    for n, tile in enumerate(tiles):
        due = (n + 1) * now / len(tiles)
        at = next((p for t, p in points if t >= due and p[1] >= tile[0]), points[-1][1])
        where.setdefault(at, []).append(tile)
    return where


def _kernel(x_hbm, wqkv_hbm, wo_hbm, wg_hbm, wu_hbm, wd_hbm, out_hbm,
            x_s, wqkv_s, wo_s, wg_s, wu_s, wd_s, wgu_s, wdp_s, xn_s, gu_s, hid_s, y_s,
            qt_s, qf_s, k_s, kh_s, kf_s, kb0_s, kb_s, vt_s, s_s, m_s, mrun_s, ot_s, o_s, out_s,
            in_sem, out_sem):
    x_copy = [pltpu.make_async_copy(x_hbm.at[pl.ds(b * TQ, TQ)], x_s.at[b], in_sem.at[b])
              for b in range(NB)]
    wq_copy, wk_copy, wv_copy = (
        pltpu.make_async_copy(wqkv_hbm.at[:, pl.ds(j * D, D)], wqkv_s.at[j], in_sem.at[NB + j])
        for j in range(3))
    late_copy = [pltpu.make_async_copy(src, dst, in_sem.at[NB + 3 + i]) for i, (src, dst) in
                 enumerate(((wg_hbm, wg_s), (wu_hbm, wu_s), (wd_hbm, wd_s), (wo_hbm, wo_s)))]
    for c in (x_copy[0], wk_copy, wq_copy, wv_copy, x_copy[1], x_copy[2], x_copy[3], *late_copy):
        c.start()

    def norm(b, during=None):
        x = x_s[b].astype(F32)
        if during is not None:
            pins = []
            for r in range(TQ // 8):
                t, o = divmod(3 * r, TQ // 8)
                pins.append(during[8 * o:8 * o + 8, t * 128:(t + 1) * 128])
            x0 = jnp.where(_never(xn_s[0, 0:8, 0:128])[None], jnp.stack(pins), _rows8(x[:, 0:128]))
            x = jnp.concatenate([x0.reshape(TQ, 128), x[:, 128:]], axis=1)
        xc = x - jnp.mean(x, axis=-1, keepdims=True)
        var = jnp.mean(xc * xc, axis=-1, keepdims=True)
        xn = pltpu.bitcast((xc * lax.rsqrt(var + 1e-5)).astype(BF16), U32)
        xn_s[b * HB:(b + 1) * HB] = xn.reshape(HB, RF // 2, D)

    def normed(b):
        return pltpu.bitcast(xn_s[b * HB:(b + 1) * HB].reshape(TQ // 2, D), BF16)

    def proj(b, j, norm_next=False):
        t = _dot(normed(b), wqkv_s[j])
        if norm_next:
            norm(b + 1, t)
        return t

    def proj_even(b, j):
        xn = normed(b)
        edge = jnp.concatenate(
            [_dot(xn[r:r + 128, WQ:], wqkv_s[j, WQ:, WQ:]) for r in range(0, TQ, 128)], axis=0)
        edge = edge + _dot(xn[:, :WQ], wqkv_s[j, :WQ, WQ:])
        return jnp.concatenate([_dot(xn, wqkv_s[j, :, :WQ]), edge], axis=1)

    def put_q(b, q):
        q = (q * QSCALE).T
        lo = lax.broadcasted_iota(jnp.int32, (8, TQ), 0) < 4
        for p in range(H // 2):
            r = 2 * DH * p
            even = [q[r:r + 16], jnp.where(lo, q[r + 16:r + 24], 0.0)]
            t = [pltpu.roll(q[i:i + 8], 4, 0) for i in range(r + 16, r + 40, 8)]
            odd = [jnp.where(lo, t[0], t[1]), jnp.where(lo, t[1], t[2]), jnp.where(lo, t[2], 0.0)]
            for h, rows in ((2 * p, even), (2 * p + 1, odd)):
                qh = jnp.concatenate(rows + [jnp.zeros((8, TQ), F32)], axis=0).astype(BF16)
                qt_s[b, h] = pltpu.bitcast(qh, U32)
                qf_s[b, h] = qh.astype(F32)[:24]

    def put_v(b, v):
        vt = v.T
        lo = lax.broadcasted_iota(jnp.int32, (8, TQ), 0) < 4
        for p in range(H // 2):
            r = 2 * DH * p
            mid = vt[r + 16:r + 24]
            vt_s[2 * p, b, 0:16] = vt[r:r + 16]
            vt_s[2 * p, b, 16:24] = jnp.where(lo, mid, 1.0)
            vt_s[2 * p + 1, b, 0:8] = jnp.where(lo, 1.0, mid)
            vt_s[2 * p + 1, b, 8:24] = vt[r + 24:r + 40]

    def put_k(b, k):
        k_s[b] = pltpu.bitcast(k.astype(BF16), U32)

    def split_heads(b):
        hi = lax.broadcasted_iota(jnp.int32, (TQ // 2, 128), 1) >= 64
        for h in range(H):
            c, lane = divmod(h * DH, 128)
            k = k_s[b, :, c * 128:(c + 1) * 128]
            if lane + DH > 128:
                k = jnp.where(hi, k, k_s[b, :, (c + 1) * 128:(c + 2) * 128])
            if lane:
                k = pltpu.roll(k, 128 - lane, 1)
            kh_s[h, b] = k
            k = jnp.concatenate([k[r:r + G // 2] for r in range(0, TQ // 2, CK // 2)], axis=0)
            kf_s[h, b] = pltpu.bitcast(k, BF16).astype(F32)

    def spread_keys(dst, h, kb, features, order=lambda k: k):
        k = order(kf_s[h, kb])
        for d in features:
            dst[d] = jnp.broadcast_to(k[:, d:d + 1], k.shape)

    def ffn_steps(i, zero, pack_weights=False):
        half_w = WQ // 2

        def gate_up(n, k):
            rows, cols = slice(k * 64, (k + 1) * 64), slice(n * WQ, (n + 1) * WQ)
            if pack_weights:
                src = slice(k * 128, (k + 1) * 128), slice(n * half_w, (n + 1) * half_w)
                w = jnp.concatenate([wg_s[src], wu_s[src]], axis=1)
                wgu_s[rows, cols] = pltpu.bitcast(w, U32)
            else:
                w = pltpu.bitcast(wgu_s[rows, cols], BF16)
            t = _dot(pltpu.bitcast(xn_s[i + zero * n, :, k * 128:(k + 1) * 128], BF16), w)
            if k > 0:
                t = t + gu_s[...]
            if k < NCH - 1:
                gu_s[...] = t
            else:
                half = t[:, :half_w] * 0.5
                gate = half * jnp.tanh(half) + half
                hid = (gate * t[:, half_w:]).astype(BF16)
                hid_s[n // 2][0, :, n % 2 * half_w:(n % 2 + 1) * half_w] = pltpu.bitcast(hid, U32)
            return t

        def down(k, n):
            rows, cols = slice(k * WQ // 2, (k + 1) * WQ // 2), slice(n * 128, (n + 1) * 128)
            if pack_weights:
                w = wd_s[k * WQ:(k + 1) * WQ, cols]
                wdp_s[rows, cols] = pltpu.bitcast(w, U32)
            else:
                w = pltpu.bitcast(wdp_s[rows, cols], BF16)
            t = _dot(pltpu.bitcast(hid_s[k][zero * n], BF16), w)
            if k > 0:
                t = t + y_s[n][i]
            y_s[n][i] = t
            return t

        return ([(gate_up, n, k) for n in range(2 * F // WQ) for k in range(NCH)]
                + [(down, k, n) for k in range(F // WQ) for n in range(NCH)])

    x_copy[0].wait()
    norm(0)
    wk_copy.wait()
    put_k(0, proj_even(0, 1))
    wq_copy.wait()
    q = proj_even(0, 0)
    wv_copy.wait()
    x_copy[1].wait()
    x_copy[2].wait()
    put_q(0, q)
    put_v(0, proj(0, 2, True))
    put_k(1, proj(1, 1, True))
    split_heads(0)
    put_q(1, proj(1, 0))
    put_v(1, proj(1, 2))
    split_heads(1)
    put_k(2, proj_even(2, 1))
    x_copy[3].wait()
    for c in late_copy:
        c.wait()
    put_q(2, proj(2, 0, True))
    split_heads(2)
    put_k(3, proj(3, 1))
    put_v(2, proj(2, 2))
    split_heads(3)
    put_q(3, proj(3, 0))
    put_v(3, proj(3, 2))
    for kb in range(NB):
        spread_keys(kb0_s.at[kb], 0, kb, range(DH))
    for kb in range(NB - 1):
        spread_keys(kb_s[kb], 1, kb, range(DH))
    for step, a, b in ffn_steps(H - 1, 0, pack_weights=True):
        step(a, b)

    def update_max(mx, s, q0):
        for t in range(s.shape[1] // 128):
            x = jnp.max(_rows8(s[:, t * 128:(t + 1) * 128]), axis=0)
            mx[q0 + t] = x if mx[q0 + t] is None else jnp.maximum(mx[q0 + t], x)

    def vpu_score(keys, h, qb, kb, c, q, mx, zero, after=None):
        cols = slice(q * 128, (q + 1) * 128)
        rows = pl.ds(pl.multiple_of(c * G + zero * (8 * (q + NT * qb)), 8), G)
        hq = h + zero * (c + CB * kb)
        s = None
        for d in range(DH):
            t = keys[d, rows, :] * qf_s[qb, hq, d:d + 1, cols]
            s = t if s is None else s + t
        if after is None:
            update_max(mx, s, q)
            s = jnp.minimum(_rows8(s), mx[q][None]).reshape(G, 128)
        else:
            s = jnp.where(zero > 0, after[None], _rows8(s)).reshape(G, 128)
            update_max(mx, s, q)
        s_s[qb, kb * TQ + c * CK:kb * TQ + c * CK + G, cols] = s

    def score(keys, h, qb, kb, c, mx, zero, where):
        k = kh_s[h + zero * qb, kb, (c * CK + G) // 2:(c + 1) * CK // 2, :]
        qt = jnp.concatenate([pltpu.bitcast(qt_s[qb, h], BF16), jnp.zeros((96, TQ), BF16)], axis=0)
        s = _dot(pltpu.bitcast(k, BF16), qt)
        s_s[qb, kb * TQ + c * CK + G:kb * TQ + (c + 1) * CK, :] = s
        for r in range(G, CK, 8):
            for tile in where.get(("score", c, r), ()):
                vpu_score(keys, h, qb, kb, *tile, mx, zero)
            update_max(mx, s[r - G:r - G + 8], 0)

    def column_max(mx):
        return jnp.broadcast_to(jnp.max(jnp.concatenate(mx, axis=1), axis=0, keepdims=True), (8, TQ))

    def probs(qb, kb, c, m):
        s = s_s[qb, kb * TQ + c * CK:kb * TQ + (c + 1) * CK, :]
        return jnp.exp2(_rows8(s) - m[None]).reshape(CK, TQ)

    def weigh(h, kb, c, p, acc):
        return acc + _dot(vt_s[h, kb, :, c * CK:(c + 1) * CK], p)

    def first_head(qb, carry):
        zero = lax.shift_right_logical(qb, 12)
        mx = [None] * NT
        for kb in range(NB):
            for c in range(CB):
                score(kb0_s.at[kb], 0, qb, kb, c, mx, zero, _tile_placement(None))
        m_s[qb] = column_max(mx)
        return carry

    lax.fori_loop(0, NB, first_head, 0)

    def head(h, carry):
        zero = lax.shift_right_logical(h, 12)
        steps = ffn_steps(h, zero)
        assert len(steps) == FFN_SLOTS.count("1") and len(FFN_SLOTS) == NB * NB * CB
        for kb in range(NB):
            for qb in range(NB):
                slot0 = (kb * NB + qb) * CB
                where = _tile_placement(slot0)
                m = m_s[qb]
                if kb == 0:
                    mx = [None] * NT
                    acc = jnp.full((24, TQ), zero.astype(F32))
                else:
                    mx = [mrun_s[qb, :, q * 128:(q + 1) * 128] for q in range(NT)]
                    acc = ot_s[qb, h]
                for c in range(CB):
                    p = probs(qb, kb, c, m)
                    score(kb_s[kb], h + 1, qb, kb, c, mx, zero, where)
                    if c == 0:
                        pin = mx[0][None]
                        spread_keys(kb_s[kb - 1], h + 1 if kb == 0 else jnp.minimum(h + 2, H - 1),
                                    (kb - 1) % NB, range(DH * qb // NB, DH * (qb + 1) // NB),
                                    lambda k: jnp.where(zero > 0, pin, _rows8(k)).reshape(k.shape))
                    acc = weigh(h + zero * qb, kb, c, p, acc)
                    if _ffn_step(slot0 + c) is not None:
                        step, a, b = steps[_ffn_step(slot0 + c)]
                        t = step(a, b)
                        for r in range(0, RF, 8):
                            for tile in where.get(("ffn", c, r), ()):
                                vpu_score(kb_s[kb], h + 1, qb, kb, *tile, mx, zero, t[r:r + 8, 0:128])
                ot_s[qb, h] = acc
                if kb < NB - 1:
                    mrun_s[qb] = jnp.concatenate(mx, axis=1)
                else:
                    m_s[qb] = column_max(mx)
        return carry

    lax.fori_loop(0, H - 1, head, 0)

    out_copy = [pltpu.make_async_copy(out_s.at[pl.ds(r, RO)], out_hbm.at[pl.ds(r, RO)], out_sem.at[r // RO])
                for r in range(0, S, RO)]
    split = -(-WQ // (2 * DH))

    def normalized(b, pairs):
        lo = lax.broadcasted_iota(jnp.int32, (8, TQ), 0) < 4
        parts = []
        for p in pairs:
            a0, a1 = ot_s[b, 2 * p], ot_s[b, 2 * p + 1]
            o0 = a0 * (1.0 / a0[20:21])
            o1 = a1 * (1.0 / a1[0:1])
            parts += [o0[0:16], jnp.where(lo, o0[16:24], o1[0:8]), o1[8:24]]
        return jnp.concatenate(parts, axis=0)

    def gather_front(b):
        o = normalized(b, range(split))[:WQ]
        o_s[b, :, :WQ] = pltpu.bitcast(o.T.astype(BF16), U32)

    def gather_back(b):
        o = normalized(b, range(split - 1, H // 2))[WQ - D:]
        o_s[b, :, WQ:] = pltpu.bitcast(o.T.astype(BF16), U32)

    def project(b, r0, r1, k0, k1, n0, n1):
        o = pltpu.bitcast(o_s[b, r0 // 2:r1 // 2, k0:k1], BF16)
        groups = slice(b * HB + r0 // RF, b * HB + r1 // RF)
        y = jnp.concatenate([y_s[n][groups].reshape(r1 - r0, 128) for n in range(n0 // 128, n1 // 128)],
                            axis=1)
        y = y + _dot(o, wo_s[k0:k1, n0:n1])
        if k1 == D:
            y = y + x_s[b, r0:r1, n0:n1].astype(F32)
            out_s[b * TQ + r0:b * TQ + r1, n0:n1] = y.astype(BF16)
        else:
            for n in range(n0 // 128, n1 // 128):
                y_s[n][groups] = y[:, n * 128 - n0:(n + 1) * 128 - n0].reshape(-1, RF, 128)

    gather_front(0)
    for b in range(NB):
        m = m_s[b]
        acc = jnp.concatenate([jnp.where(_never(qt_s[b, 0, 0:8, :]), m, 0.0)] * 3, axis=0)
        for kb in range(NB):
            for c in range(CB):
                project(b, 128 * c, 128 * c + 128, 128 * kb, 128 * kb + 128, 0, WQ)
                acc = weigh(H - 1, kb, c, probs(b, kb, c, m), acc)
        ot_s[b, H - 1] = acc
        gather_back(b)
        if b + 1 < NB:
            gather_front(b + 1)
        project(b, 0, TQ, 0, WQ, WQ, D)
        for r in range(0, TQ, 128):
            project(b, r, r + 128, WQ, D, WQ, D)
        for r in range(0, TQ, RO):
            project(b, r, r + RO, WQ, D, 0, WQ)
            out_copy[(b * TQ + r) // RO].start()
    for c in out_copy:
        c.wait()


@jax.jit
def pallas_parallel_sum__mha_block__swiglu_ffn__prompt_kernel(
    A_x: jax.Array,
    A_wqkv: jax.Array,
    A_wo: jax.Array,
    B_x: jax.Array,
    B_w_gate: jax.Array,
    B_w_up: jax.Array,
    B_w_down: jax.Array,
):
    del B_x
    hbm = pl.BlockSpec(memory_space=pl.ANY)
    vmem = pltpu.VMEM
    out = pl.pallas_call(
        _kernel,
        out_shape=jax.ShapeDtypeStruct((S, D), BF16),
        in_specs=[hbm] * 6,
        out_specs=hbm,
        scratch_shapes=[
            vmem((NB, TQ, D), BF16),
            vmem((3, D, D), BF16),
            vmem((D, D), BF16),
            vmem((D, F), BF16),
            vmem((D, F), BF16),
            vmem((F, D), BF16),
            vmem((D // 2, 2 * F), U32),
            vmem((F // 2, D), U32),
            vmem((H, RF // 2, D), U32),
            vmem((RF, WQ), F32),
            [vmem((1, RF // 2, WQ), U32)] * (F // WQ),
            [vmem((H, RF, 128), F32)] * NCH,
            vmem((NB, H, 16, TQ), U32),
            vmem((NB, H, 24, TQ), F32),
            vmem((NB, TQ // 2, D), U32),
            vmem((H, NB, TQ // 2, 128), U32),
            vmem((H, NB, CB * G, 128), F32),
            vmem((NB, DH, CB * G, 128), F32),
            [vmem((DH, CB * G, 128), F32)] * NB,
            vmem((H, NB, 24, TQ), F32),
            vmem((NB, S, TQ), F32),
            vmem((NB, 8, TQ), F32),
            vmem((NB, 8, TQ), F32),
            vmem((NB, H, 24, TQ), F32),
            vmem((NB, TQ // 2, D), U32),
            vmem((S, D), BF16),
            pltpu.SemaphoreType.DMA((NB + 7,)),
            pltpu.SemaphoreType.DMA((S // RO,)),
        ],
        compiler_params=pltpu.CompilerParams(vmem_limit_bytes=112 << 20),
        name="fused_block",
    )(A_x.reshape(S, D), A_wqkv, A_wo, B_w_gate, B_w_up, B_w_down)
    return out.reshape(1, S, D)
```
